```python
import os as _os
_os.environ.setdefault("JAX_PLATFORMS", "cpu")
import jax
import jax.numpy as jnp

def _softmax(x, axis=-1):
    return jax.nn.softmax(x, axis=axis)
def _gelu(x):
    return jax.nn.gelu(x, approximate=True)
def _silu(x):
    return jax.nn.silu(x)
def _sigmoid(x):
    return jax.nn.sigmoid(x)
def _layernorm(x, axis=-1, eps=1e-5):
    m = jnp.mean(x, axis=axis, keepdims=True)
    v = jnp.var(x, axis=axis, keepdims=True)
    return (x - m) / jnp.sqrt(v + eps)
def _scatter_add(tgt, idx, src, axis=0):
    return tgt.at[idx].add(src)
def _segment_sum(src, seg, n):
    return jax.ops.segment_sum(src, seg, n)
class _Rng:
    def __init__(self, key):
        self._k = key
    def _next(self):
        self._k, sub = jax.random.split(self._k)
        return sub
    def normal(self, shape):
        return jax.random.normal(self._next(), shape, dtype=jnp.bfloat16)
    def randint(self, lo, hi, shape):
        return jax.random.randint(self._next(), shape, lo, hi, dtype=jnp.int32)
    def uniform(self, shape, lo=0.0, hi=1.0):
        return jax.random.uniform(self._next(), shape, jnp.bfloat16, lo, hi)
    def permutation(self, n):
        return jax.random.permutation(self._next(), n)


kernel_name = 'sequential_preLN__compressed_kv_cla__dense_activation_mish__decode'

def setup_inputs():
    _rng = _Rng(jax.random.key(int.from_bytes(__import__("os").urandom(4), "little")))
    _w = (lambda a: (lambda t: t.astype(jnp.bfloat16) if jnp.issubdtype(t.dtype, jnp.floating) else t)(jnp.asarray(a)))
    def _A_setup():
        B, H, Sq, Sk, D, M = 2, 32, 1, 8192, 128, 512
        Dc = 4 * D
        return {
            "x": _w((lambda *s: _rng.normal(s) * 0.05)(B, Sq, M)),
            "c_kv": _w((lambda *s: _rng.normal(s) * 0.8)(B, Sk, Dc)),
            "w_q": _w((lambda *s: _rng.normal(s) * 0.8)(M, H, D) * (M ** -0.5)),
            "w_uk": _w((lambda *s: _rng.normal(s) * 0.8)(Dc, H, D) * (Dc ** -0.5)),
            "w_uv": _w((lambda *s: _rng.normal(s) * 0.8)(Dc, H, D) * (Dc ** -0.5)),
            "w_o": _w((lambda *s: _rng.normal(s) * 0.8)(H, D, M) * ((H * D) ** -0.5)),
        }
    _A_in = _A_setup()

    def _B_setup():
        B, S, D, F = 2, 1, 512, 1792
        return {
            "x": _w((lambda *s: _rng.normal(s) * 0.05)(B, S, D)),
            "w1": _w((lambda *s: _rng.normal(s) * 0.4)(D, F) * (D ** -0.5)),
            "b1": _w((lambda *s: _rng.normal(s) * 0.05)(F)),
            "w2": _w((lambda *s: _rng.normal(s) * 0.05)(F, D) * (F ** -0.5)),
        }
    _B_in = _B_setup()

    return {
        "A_x": _A_in["x"],
        "A_c_kv": _A_in["c_kv"],
        "A_w_q": _A_in["w_q"],
        "A_w_uk": _A_in["w_uk"],
        "A_w_uv": _A_in["w_uv"],
        "A_w_o": _A_in["w_o"],
        "B_x": _B_in["x"],
        "B_w1": _B_in["w1"],
        "B_b1": _B_in["b1"],
        "B_w2": _B_in["w2"],
    }

def reference(A_x, A_c_kv, A_w_q, A_w_uk, A_w_uv, A_w_o, B_x, B_w1, B_b1, B_w2):
    def _A_ref(x, c_kv, w_q, w_uk, w_uv, w_o):
        B, Sq, M = x.shape[0], x.shape[1], x.shape[2]
        Sk = c_kv.shape[1]
        H, D = w_q.shape[1], w_q.shape[2]
        q = jnp.einsum("bqm,mhd->bhqd", x, w_q)
        k = jnp.einsum("bkc,chd->bhkd", c_kv, w_uk)
        v = jnp.einsum("bkc,chd->bhkd", c_kv, w_uv)
        scores = jnp.einsum("bhqd,bhkd->bhqk", q, k) * (D ** -0.5)
        off = Sk - Sq
        qi = jnp.arange(Sq)[:, None]
        kj = jnp.arange(Sk)[None, :]
        cmask = kj <= (qi + off)
        scores = jnp.where(cmask[None, None], scores, -1e9)
        p = _softmax(scores, axis=-1)
        ctx = jnp.einsum("bhqk,bhkd->bhqd", p, v)
        return jnp.einsum("bhqd,hdm->bqm", ctx, w_o)

    def _B_ref(x, w1, b1, w2):
        h = jnp.einsum("bsd,df->bsf", x, w1) + b1
        sp = jnp.log1p(jnp.exp(-jnp.abs(h))) + jnp.where(h > 0, h, jnp.zeros_like(h))
        act = h * jnp.tanh(sp)
        return jnp.einsum("bsf,fd->bsd", act, w2)

    x = A_x
    h = x + _A_ref(_layernorm(x, axis=-1), A_c_kv, A_w_q, A_w_uk, A_w_uv, A_w_o)
    h2 = h + _B_ref(_layernorm(h, axis=-1), B_w1, B_b1, B_w2)
    return h2
```

```python
import functools
import numpy as np
import jax
import jax.numpy as jnp
from jax import lax
import jax.experimental.pallas as pl
import jax.experimental.pallas.tpu as pltpu

f32, bf16, i32 = jnp.float32, jnp.bfloat16, jnp.int32
NT = (((1,), (1,)), ((), ()))
B, H, D, M, SK, DC, F = 2, 32, 128, 512, 8192, 512, 1792
CH = 2048
NCH = SK // CH
W2_CHUNKS = (1280, 256, 128, 128)
VPU_TAIL = True
import contextlib


def scope(name):
    return contextlib.nullcontext()


def _ln(x):
    m = jnp.mean(x, axis=-1, keepdims=True)
    xc = x - m
    v = jnp.mean(xc * xc, axis=-1, keepdims=True)
    return xc * lax.rsqrt(v + 1e-5)


def _expand_blockdiag(a_u, lane, row_h):
    keep = (lane % 32) == row_h
    parts = []
    for t in range(32):
        idx = 4 * t + lane // 32
        g = jnp.take_along_axis(a_u, idx, axis=1)
        parts.append(jnp.where(keep, g, 0.0).astype(bf16))
    return jnp.concatenate(parts, axis=1)


def _head_contract(a, w_ref, lane, row_h):
    acc = jnp.zeros((64, 128), f32)
    for u in range(4):
        L = _expand_blockdiag(a[:, u * 128:(u + 1) * 128], lane, row_h)
        acc = acc + jnp.dot(L, w_ref[pl.ds(u * 4096, 4096), :], preferred_element_type=f32)
    return acc


def kernel(x_hbm, wq_hbm, wuk_hbm, ckv_hbm, wuv_hbm, wo_hbm, w1_hbm, b1_hbm, w2_hbm,
           o_ref,
           x_v, wq_v, wuk_v, ckv_v, wuv_v, wo_v, w1_v, b1_v, w2_v, ql_v):
    NS = 2 * NCH
    NW2 = len(W2_CHUNKS)
    w2_off = [sum(W2_CHUNKS[:i]) for i in range(NW2)]

    def main(sems):
        def cp_w2(i):
            return pltpu.make_async_copy(w2_hbm.at[pl.ds(w2_off[i], W2_CHUNKS[i])], w2_v.at[pl.ds(w2_off[i], W2_CHUNKS[i])], sems.at[7 + NS + i])
        cp_x = pltpu.make_async_copy(x_hbm, x_v, sems.at[0])
        cp_wq = pltpu.make_async_copy(wq_hbm, wq_v, sems.at[1])
        cp_wuk = pltpu.make_async_copy(wuk_hbm, wuk_v, sems.at[2])
        def cp_ckv(i):
            return pltpu.make_async_copy(ckv_hbm.at[pl.ds(i * CH, CH)], ckv_v.at[pl.ds(i * CH, CH)], sems.at[3 + i])
        cp_wuv = pltpu.make_async_copy(wuv_hbm, wuv_v, sems.at[3 + NS])
        cp_wo = pltpu.make_async_copy(wo_hbm, wo_v, sems.at[4 + NS])
        cp_w1 = pltpu.make_async_copy(w1_hbm, w1_v, sems.at[5 + NS])
        cp_b1 = pltpu.make_async_copy(b1_hbm, b1_v, sems.at[6 + NS])

        with scope("issue"):
            cp_wq.start()
            cp_x.start()
            cp_wuk.start()
            for i in range(NS):
                cp_ckv(i).start()
            cp_wuv.start()
            cp_wo.start()
            cp_b1.start()
            cp_w1.start()
            for i in range(NW2):
                cp_w2(i).start()

        lane = lax.broadcasted_iota(i32, (64, 128), 1)
        row = lax.broadcasted_iota(i32, (64, 128), 0)
        row_h = row % 32

        with scope("wait_wq"):
            cp_x.wait()
            cp_wq.wait()
        with scope("phase1"):
            x = x_v[...].astype(f32)
            xn = _ln(x).astype(bf16).astype(f32)
            row512 = lax.broadcasted_iota(i32, (64, 512), 0)
            a1 = jnp.where(row512 < 32, xn[0:1, :], xn[1:2, :])
            q = _head_contract(a1, wq_v, lane, row_h)
            qb = q.astype(bf16)
        with scope("wait_wuk"):
            cp_wuk.wait()
        with scope("phase2"):
            gidx = (lane % 4) * 32 + row_h
            scale = (D ** -0.5) * np.log2(np.e)
            for u in range(4):
                out = lax.dot_general(qb, wuk_v[pl.ds(u * 4096, 4096), :], NT, preferred_element_type=f32)
                dest = jnp.zeros((64, 128), f32)
                for t in range(32):
                    g = jnp.take_along_axis(out[:, t * 128:(t + 1) * 128], gidx, axis=1)
                    dest = jnp.where(lane // 4 == t, g, dest)
                ql_v[:, pl.ds(u * 128, 128)] = (dest * scale).astype(bf16)

        ctx_lat = []
        for b in range(B):
            qb_lat = ql_v[pl.ds(b * 32, 32), :]
            m = jnp.full((32, 1), -jnp.inf, f32)
            l = jnp.zeros((32, 1), f32)
            acc = jnp.zeros((32, 512), f32)
            for j in range(NCH):
                i = b * NCH + j
                with scope(f"wait_ckv{i}"):
                    cp_ckv(i).wait()
                with scope(f"att{i}"):
                    c = ckv_v[pl.ds(i * CH, CH), :]
                    s = lax.dot_general(qb_lat, c, NT, preferred_element_type=f32)
                    m_new = jnp.maximum(m, jnp.max(s, axis=1, keepdims=True))
                    alpha = jnp.exp2(m - m_new)
                    p = jnp.exp2(s - m_new)
                    l = l * alpha + jnp.sum(p, axis=1, keepdims=True)
                    acc = acc * alpha + jnp.dot(p.astype(bf16), c, preferred_element_type=f32)
                    m = m_new
            ctx_lat.append(acc / l)
        with scope("wait_wuv"):
            cp_wuv.wait()
        with scope("phase4"):
            a4 = jnp.concatenate(ctx_lat, axis=0).astype(bf16).astype(f32)
            ctx = _head_contract(a4, wuv_v, lane, row_h)
        with scope("wait_wo"):
            cp_wo.wait()
        with scope("phase5"):
            sub = lax.broadcasted_iota(i32, (8, 128), 0)
            pieces = []
            for hh in range(32):
                r0 = ctx[hh:hh + 1, :]
                r1 = ctx[32 + hh:33 + hh, :]
                pieces.append(jnp.where(sub == 0, r0, r1))
            L5 = jnp.concatenate(pieces, axis=1).astype(bf16)
            att = jnp.dot(L5, wo_v[...], preferred_element_type=f32)[0:2, :]
            h = x + att
            hn = _ln(h).astype(bf16)
        with scope("wait_w1"):
            cp_w1.wait()
            cp_b1.wait()
        with scope("phase6"):
            h1 = jnp.dot(hn, w1_v[...], preferred_element_type=f32)
            bb = b1_v[...].astype(f32)
            h1 = jnp.concatenate([h1[:, j * 128:(j + 1) * 128] + bb[j:j + 1, :] for j in range(F // 128)], axis=1)
            sp = jnp.log1p(jnp.exp(-jnp.abs(h1))) + jnp.maximum(h1, 0.0)
            act = (h1 * jnp.tanh(sp)).astype(bf16)
            if VPU_TAIL:
                R = W2_CHUNKS[-1]
                al = act[:, w2_off[-1]:].astype(f32)
                ident = (lax.broadcasted_iota(i32, (R, R), 0) == lax.broadcasted_iota(i32, (R, R), 1))
                acol = []
                for b in range(B):
                    d = jnp.where(ident, al[b:b + 1, :], 0.0)
                    acol.append(jnp.broadcast_to(jnp.sum(d, axis=1, keepdims=True), (R, 128)))
        y = h
        for i in range(NW2 - 1 if VPU_TAIL else NW2):
            with scope(f"wait_w2_{i}"):
                cp_w2(i).wait()
            with scope(f"phase7_{i}"):
                y = y + jnp.dot(act[:, w2_off[i]:w2_off[i] + W2_CHUNKS[i]], w2_v[pl.ds(w2_off[i], W2_CHUNKS[i]), :], preferred_element_type=f32)
        if VPU_TAIL:
            with scope(f"wait_w2_last"):
                cp_w2(NW2 - 1).wait()
            with scope(f"phase7_last"):
                wl = w2_v[pl.ds(w2_off[-1], R), :].astype(f32)
                outs = []
                for b in range(B):
                    cols = []
                    for n in range(4):
                        cols.append(jnp.sum(acol[b] * wl[:, n * 128:(n + 1) * 128], axis=0, keepdims=True))
                    outs.append(jnp.concatenate(cols, axis=1))
                sub2 = lax.broadcasted_iota(i32, (2, 512), 0)
                y = y + jnp.where(sub2 == 0, outs[0], outs[1])
        o_ref[...] = y.astype(bf16)

    pl.run_scoped(main, pltpu.SemaphoreType.DMA((7 + NS + NW2,)))


@jax.jit
def pallas_sequential_preLN__compressed_kv_cla__dense_activation_mish__decode_kernel(A_x, A_c_kv, A_w_q, A_w_uk, A_w_uv, A_w_o, B_x, B_w1, B_b1, B_w2):
    anys = pl.BlockSpec(memory_space=pl.ANY)
    out = pl.pallas_call(
        kernel,
        out_shape=jax.ShapeDtypeStruct((B, M), bf16),
        in_specs=[anys] * 9,
        out_specs=pl.BlockSpec(memory_space=pltpu.VMEM),
        scratch_shapes=[
            pltpu.VMEM((B, M), bf16),
            pltpu.VMEM((M * H, D), bf16),
            pltpu.VMEM((DC * H, D), bf16),
            pltpu.VMEM((B * SK, DC), bf16),
            pltpu.VMEM((DC * H, D), bf16),
            pltpu.VMEM((H * D, M), bf16),
            pltpu.VMEM((M, F), bf16),
            pltpu.VMEM((F // 128, 128), bf16),
            pltpu.VMEM((F, M), bf16),
            pltpu.VMEM((64, DC), bf16),
        ],
        compiler_params=pltpu.CompilerParams(vmem_limit_bytes=100 * 1024 * 1024),
    )(A_x.reshape(B, M), A_w_q.reshape(M * H, D), A_w_uk.reshape(DC * H, D), A_c_kv.reshape(B * SK, DC),
      A_w_uv.reshape(DC * H, D), A_w_o.reshape(H * D, M), B_w1, B_b1.reshape(F // 128, 128), B_w2)
    return out.reshape(B, 1, M)
```

```python
import functools
import numpy as np
import jax
import jax.numpy as jnp
from jax import lax
import jax.experimental.pallas as pl
import jax.experimental.pallas.tpu as pltpu

f32, bf16, i32 = jnp.float32, jnp.bfloat16, jnp.int32
NT = (((1,), (1,)), ((), ()))
B, H, D, M, SK, DC, F = 2, 32, 128, 512, 8192, 512, 1792
CH = 2048
NCH = SK // CH
W2_MXU = (1152, 384, 128)
W2_VPU = (64, 64)
W2_CHUNKS = W2_MXU + W2_VPU
VPU_TAIL = True
import contextlib
SCOPES = False
def scope(name):
    return jax.named_scope(name) if SCOPES else contextlib.nullcontext()


def _ln(x):
    m = jnp.mean(x, axis=-1, keepdims=True)
    xc = x - m
    v = jnp.mean(xc * xc, axis=-1, keepdims=True)
    return xc * lax.rsqrt(v + 1e-5)


def _expand_blockdiag(a_u, lane, row_h):
    keep = (lane % 32) == row_h
    parts = []
    for t in range(32):
        idx = 4 * t + lane // 32
        g = jnp.take_along_axis(a_u, idx, axis=1)
        parts.append(jnp.where(keep, g, 0.0).astype(bf16))
    return jnp.concatenate(parts, axis=1)


def _head_contract(a, w_ref, lane, row_h):
    acc = jnp.zeros((64, 128), f32)
    for u in range(4):
        L = _expand_blockdiag(a[:, u * 128:(u + 1) * 128], lane, row_h)
        acc = acc + jnp.dot(L, w_ref[pl.ds(u * 4096, 4096), :], preferred_element_type=f32)
    return acc


def kernel(x_hbm, wq_hbm, wuk_hbm, ckv_hbm, wuv_hbm, wo_hbm, w1_hbm, b1_hbm, w2_hbm,
           o_ref,
           x_v, wq_v, wuk_v, ckv_v, wuv_v, wo_v, w1_v, b1_v, w2_v, ql_v):
    NS = 2 * NCH
    NW2 = len(W2_CHUNKS)
    w2_off = [sum(W2_CHUNKS[:i]) for i in range(NW2)]

    def main(sems):
        def cp_w2(i):
            return pltpu.make_async_copy(w2_hbm.at[pl.ds(w2_off[i], W2_CHUNKS[i])], w2_v.at[pl.ds(w2_off[i], W2_CHUNKS[i])], sems.at[7 + NS + i])
        cp_x = pltpu.make_async_copy(x_hbm, x_v, sems.at[0])
        cp_wq = pltpu.make_async_copy(wq_hbm, wq_v, sems.at[1])
        cp_wuk = pltpu.make_async_copy(wuk_hbm, wuk_v, sems.at[2])
        def cp_ckv(i):
            return pltpu.make_async_copy(ckv_hbm.at[pl.ds(i * CH, CH)], ckv_v.at[pl.ds(i * CH, CH)], sems.at[3 + i])
        cp_wuv = pltpu.make_async_copy(wuv_hbm, wuv_v, sems.at[3 + NS])
        cp_wo = pltpu.make_async_copy(wo_hbm, wo_v, sems.at[4 + NS])
        cp_w1 = pltpu.make_async_copy(w1_hbm, w1_v, sems.at[5 + NS])
        cp_b1 = pltpu.make_async_copy(b1_hbm, b1_v, sems.at[6 + NS])

        with scope("issue"):
            cp_wq.start()
            cp_x.start()
            cp_wuk.start()
            for i in range(NS):
                cp_ckv(i).start()
            cp_wuv.start()
            cp_wo.start()
            cp_b1.start()
            cp_w1.start()
            for i in range(NW2):
                cp_w2(i).start()

        lane = lax.broadcasted_iota(i32, (64, 128), 1)
        row = lax.broadcasted_iota(i32, (64, 128), 0)
        row_h = row % 32

        with scope("wait_wq"):
            cp_x.wait()
            cp_wq.wait()
        with scope("phase1"):
            x = x_v[...].astype(f32)
            xn = _ln(x).astype(bf16).astype(f32)
            row512 = lax.broadcasted_iota(i32, (64, 512), 0)
            a1 = jnp.where(row512 < 32, xn[0:1, :], xn[1:2, :])
            q = _head_contract(a1, wq_v, lane, row_h)
            qb = q.astype(bf16)
        with scope("wait_wuk"):
            cp_wuk.wait()
        with scope("phase2"):
            gidx = (lane % 4) * 32 + row_h
            scale = (D ** -0.5) * np.log2(np.e)
            for u in range(4):
                out = lax.dot_general(qb, wuk_v[pl.ds(u * 4096, 4096), :], NT, preferred_element_type=f32)
                dest = jnp.zeros((64, 128), f32)
                for t in range(32):
                    g = jnp.take_along_axis(out[:, t * 128:(t + 1) * 128], gidx, axis=1)
                    dest = jnp.where(lane // 4 == t, g, dest)
                ql_v[:, pl.ds(u * 128, 128)] = (dest * scale).astype(bf16)

        ctx_lat = []
        for b in range(B):
            qb_lat = ql_v[pl.ds(b * 32, 32), :]
            m = jnp.full((32, 1), -jnp.inf, f32)
            l = jnp.zeros((32, 1), f32)
            acc = jnp.zeros((32, 512), f32)
            for j in range(NCH):
                i = b * NCH + j
                with scope(f"wait_ckv{i}"):
                    cp_ckv(i).wait()
                with scope(f"att{i}"):
                    c = ckv_v[pl.ds(i * CH, CH), :]
                    s = lax.dot_general(qb_lat, c, NT, preferred_element_type=f32)
                    m_new = jnp.maximum(m, jnp.max(s, axis=1, keepdims=True))
                    alpha = jnp.exp2(m - m_new)
                    p = jnp.exp2(s - m_new)
                    l = l * alpha + jnp.sum(p, axis=1, keepdims=True)
                    acc = acc * alpha + jnp.dot(p.astype(bf16), c, preferred_element_type=f32)
                    m = m_new
            ctx_lat.append(acc / l)
        with scope("wait_wuv"):
            cp_wuv.wait()
        with scope("phase4"):
            a4 = jnp.concatenate(ctx_lat, axis=0).astype(bf16).astype(f32)
            ctx = _head_contract(a4, wuv_v, lane, row_h)
        with scope("wait_wo"):
            cp_wo.wait()
        with scope("phase5"):
            sub = lax.broadcasted_iota(i32, (8, 128), 0)
            pieces = []
            for hh in range(32):
                r0 = ctx[hh:hh + 1, :]
                r1 = ctx[32 + hh:33 + hh, :]
                pieces.append(jnp.where(sub == 0, r0, r1))
            L5 = jnp.concatenate(pieces, axis=1).astype(bf16)
            att = jnp.dot(L5, wo_v[...], preferred_element_type=f32)[0:2, :]
            h = x + att
            hn = _ln(h).astype(bf16)
        with scope("wait_w1"):
            cp_w1.wait()
            cp_b1.wait()
        with scope("phase6"):
            h1 = jnp.dot(hn, w1_v[...], preferred_element_type=f32)
            bb = b1_v[...].astype(f32)
            h1 = jnp.concatenate([h1[:, j * 128:(j + 1) * 128] + bb[j:j + 1, :] for j in range(F // 128)], axis=1)
            sp = jnp.log1p(jnp.exp(-jnp.abs(h1))) + jnp.maximum(h1, 0.0)
            act = (h1 * jnp.tanh(sp)).astype(bf16)
            R = sum(W2_VPU)
            v0 = F - R
            al = act[:, v0:].astype(f32)
            RP = 128
            alp = jnp.concatenate([al, jnp.zeros((2, RP - R), f32)], axis=1) if R < RP else al
            ident = (lax.broadcasted_iota(i32, (R, RP), 0) == lax.broadcasted_iota(i32, (R, RP), 1))
            acol = []
            for b in range(B):
                d = jnp.where(ident, alp[b:b + 1, :], 0.0)
                acol.append(jnp.broadcast_to(jnp.sum(d, axis=1, keepdims=True), (R, 128)))
        y = h
        for i in range(len(W2_MXU)):
            with scope(f"wait_w2_{i}"):
                cp_w2(i).wait()
            with scope(f"phase7_{i}"):
                y = y + jnp.dot(act[:, w2_off[i]:w2_off[i] + W2_CHUNKS[i]], w2_v[pl.ds(w2_off[i], W2_CHUNKS[i]), :], preferred_element_type=f32)
        accs = [[None] * 4 for _ in range(B)]
        for i in range(len(W2_MXU), NW2):
            with scope(f"wait_w2_{i}"):
                cp_w2(i).wait()
            with scope(f"phase7_{i}"):
                for g in range(W2_CHUNKS[i] // 16):
                    r0 = w2_off[i] + g * 16
                    for n in range(4):
                        wv = w2_v[pl.ds(r0, 16), pl.ds(n * 128, 128)].astype(f32)
                        for b in range(B):
                            pr = acol[b][r0 - v0:r0 - v0 + 16, :] * wv
                            pr = pr[0:8, :] + pr[8:16, :]
                            accs[b][n] = pr if accs[b][n] is None else accs[b][n] + pr
        sub2 = lax.broadcasted_iota(i32, (2, 512), 0)
        outs = [jnp.concatenate([jnp.sum(accs[b][n], axis=0, keepdims=True) for n in range(4)], axis=1) for b in range(B)]
        y = y + jnp.where(sub2 == 0, outs[0], outs[1])
        o_ref[...] = y.astype(bf16)

    pl.run_scoped(main, pltpu.SemaphoreType.DMA((7 + NS + NW2,)))


@jax.jit
def pallas_sequential_preLN__compressed_kv_cla__dense_activation_mish__decode_kernel(A_x, A_c_kv, A_w_q, A_w_uk, A_w_uv, A_w_o, B_x, B_w1, B_b1, B_w2):
    anys = pl.BlockSpec(memory_space=pl.ANY)
    out = pl.pallas_call(
        kernel,
        out_shape=jax.ShapeDtypeStruct((B, M), bf16),
        in_specs=[anys] * 9,
        out_specs=pl.BlockSpec(memory_space=pltpu.VMEM),
        scratch_shapes=[
            pltpu.VMEM((B, M), bf16),
            pltpu.VMEM((M * H, D), bf16),
            pltpu.VMEM((DC * H, D), bf16),
            pltpu.VMEM((B * SK, DC), bf16),
            pltpu.VMEM((DC * H, D), bf16),
            pltpu.VMEM((H * D, M), bf16),
            pltpu.VMEM((M, F), bf16),
            pltpu.VMEM((F // 128, 128), bf16),
            pltpu.VMEM((F, M), bf16),
            pltpu.VMEM((64, DC), bf16),
        ],
        compiler_params=pltpu.CompilerParams(vmem_limit_bytes=56 * 1024 * 1024),
    )(A_x.reshape(B, M), A_w_q.reshape(M * H, D), A_w_uk.reshape(DC * H, D), A_c_kv.reshape(B * SK, DC),
      A_w_uv.reshape(DC * H, D), A_w_o.reshape(H * D, M), B_w1, B_b1.reshape(F // 128, 128), B_w2)
    return out.reshape(B, 1, M)
```
